```python
import os as _os
_os.environ.setdefault("JAX_PLATFORMS", "cpu")
import jax
import jax.numpy as jnp

def _softmax(x, axis=-1):
    return jax.nn.softmax(x, axis=axis)
def _gelu(x):
    return jax.nn.gelu(x, approximate=True)
def _silu(x):
    return jax.nn.silu(x)
def _sigmoid(x):
    return jax.nn.sigmoid(x)
def _layernorm(x, axis=-1, eps=1e-5):
    m = jnp.mean(x, axis=axis, keepdims=True)
    v = jnp.var(x, axis=axis, keepdims=True)
    return (x - m) / jnp.sqrt(v + eps)
def _scatter_add(tgt, idx, src, axis=0):
    return tgt.at[idx].add(src)
def _segment_sum(src, seg, n):
    return jax.ops.segment_sum(src, seg, n)
class _Rng:
    def __init__(self, key):
        self._k = key
    def _next(self):
        self._k, sub = jax.random.split(self._k)
        return sub
    def normal(self, shape):
        return jax.random.normal(self._next(), shape, dtype=jnp.bfloat16)
    def randint(self, lo, hi, shape):
        return jax.random.randint(self._next(), shape, lo, hi, dtype=jnp.int32)
    def uniform(self, shape, lo=0.0, hi=1.0):
        return jax.random.uniform(self._next(), shape, jnp.bfloat16, lo, hi)
    def permutation(self, n):
        return jax.random.permutation(self._next(), n)


kernel_name = 'interleave_layers__gqa_block_cached__dense_activation_mish__decode'

def setup_inputs():
    _rng = _Rng(jax.random.key(int.from_bytes(__import__("os").urandom(4), "little")))
    _w = (lambda a: (lambda t: t.astype(jnp.bfloat16) if jnp.issubdtype(t.dtype, jnp.floating) else t)(jnp.asarray(a)))
    def _A_setup():
        B, Sq, D = 1, 1, 512
        Hq, Hkv, Sk, Dh = 32, 8, 65536, 128
        assert Hq % Hkv == 0, (Hq, Hkv)
        return {
            "x": _w((lambda *s: _rng.normal(s) * 0.05)(B, Sq, D)),
            "k_cache": _w((lambda *s: _rng.normal(s) * 1.6)(B, Hkv, Sk, Dh)),
            "v_cache": _w((lambda *s: _rng.normal(s) * 1.6)(B, Hkv, Sk, Dh)),
            "wq": _w((lambda *s: _rng.normal(s) * 1.6)(D, Hq * Dh) * (D ** -0.5)),
            "wo": _w((lambda *s: _rng.normal(s) * 1.6)(Hq * Dh, D) * ((Hq * Dh) ** -0.5)),
        }
    _A_in = _A_setup()

    def _B_setup():
        B, S, D, F = 1, 1, 512, 1792
        return {
            "x": _w((lambda *s: _rng.normal(s) * 0.05)(B, S, D)),
            "w1": _w((lambda *s: _rng.normal(s) * 0.8)(D, F) * (D ** -0.5)),
            "b1": _w((lambda *s: _rng.normal(s) * 0.8)(F)),
            "w2": _w((lambda *s: _rng.normal(s) * 0.8)(F, D) * (F ** -0.5)),
        }
    _B_in = _B_setup()

    return {
        "A_x": _A_in["x"],
        "A_k_cache": _A_in["k_cache"],
        "A_v_cache": _A_in["v_cache"],
        "A_wq": _A_in["wq"],
        "A_wo": _A_in["wo"],
        "B_x": _B_in["x"],
        "B_w1": _B_in["w1"],
        "B_b1": _B_in["b1"],
        "B_w2": _B_in["w2"],
    }

def reference(A_x, A_k_cache, A_v_cache, A_wq, A_wo, B_x, B_w1, B_b1, B_w2):
    def _A_ref(x, k_cache, v_cache, wq, wo):
        B, Sq, D = x.shape
        Hq, Dh = 32, 128
        Hkv = k_cache.shape[1]
        rep = Hq // Hkv
        q = (lambda x, *d: x.transpose(*d))((x @ wq).reshape(B, Sq, Hq, Dh), 0, 2, 1, 3)
        k = jnp.repeat(k_cache, rep, axis=1)
        v = jnp.repeat(v_cache, rep, axis=1)
        scores = jnp.einsum("bhqd,bhkd->bhqk", q, k) * (Dh ** -0.5)
        p = _softmax(scores, axis=-1)
        o = jnp.einsum("bhqk,bhkd->bhqd", p, v)
        return (lambda x, *d: x.transpose(*d))(o, 0, 2, 1, 3).reshape(B, Sq, Hq * Dh) @ wo

    def _B_ref(x, w1, b1, w2):
        h = jnp.einsum("bsd,df->bsf", x, w1) + b1
        sp = jnp.log1p(jnp.exp(-jnp.abs(h))) + jnp.where(h > 0, h, jnp.zeros_like(h))
        act = h * jnp.tanh(sp)
        return jnp.einsum("bsf,fd->bsd", act, w2)

    x = A_x
    x = x + _A_ref(_layernorm(x, axis=-1), A_k_cache, A_v_cache, A_wq, A_wo)
    x = x + _B_ref(_layernorm(x, axis=-1), B_w1, B_b1, B_w2)
    x = x + _A_ref(_layernorm(x, axis=-1), A_k_cache, A_v_cache, A_wq, A_wo)
    x = x + _B_ref(_layernorm(x, axis=-1), B_w1, B_b1, B_w2)
    return x
```

```python
import functools
import jax
import jax.numpy as jnp
import numpy as np
from jax import lax
from jax.experimental import pallas as pl
from jax.experimental.pallas import tpu as pltpu

_D = 512
_HQ = 32
_HKV = 8
_DH = 128
_F = 1792
_SK = 65536


def _layernorm(x):
    m = jnp.mean(x, axis=-1, keepdims=True)
    xc = x - m
    v = jnp.mean(xc * xc, axis=-1, keepdims=True)
    return xc / jnp.sqrt(v + 1e-5)


def make_kernel(SB=256, N=116, NS=4, RHO=2, DHB=2, DSB=64, UNROLL=1):
    T = _SK // SB
    ND = T - N
    descs = [(a, b) for b in range(SB // DSB) for a in range(_HKV // DHB)]
    nt = (((1,), (1,)), ((), ()))
    scale = float(_DH) ** -0.5

    def kernel(x_hbm, k_hbm, v_hbm, wq_hbm, wo_hbm, w1_hbm, b1_hbm, w2_hbm,
               o_ref,
               kbuf, vbuf, wq_v, wo_v, w1_v, w2_v, b1_v, x_v, q_scr, kvsem, wsem):

        def start(blk, slot, si):
            s0 = blk * SB
            for (a, b) in descs:
                pltpu.make_async_copy(
                    k_hbm.at[pl.ds(a * DHB, DHB), pl.ds(s0 + b * DSB, DSB)],
                    kbuf.at[slot, pl.ds(a * DHB, DHB), pl.ds(b * DSB, DSB)],
                    kvsem.at[0, si]).start(priority=0)
                pltpu.make_async_copy(
                    v_hbm.at[pl.ds(a * DHB, DHB), pl.ds(s0 + b * DSB, DSB)],
                    vbuf.at[slot, pl.ds(a * DHB, DHB), pl.ds(b * DSB, DSB)],
                    kvsem.at[1, si]).start(priority=1)

        def wait(slot, si):
            pltpu.make_async_copy(kbuf.at[slot], kbuf.at[slot], kvsem.at[0, si]).wait()
            pltpu.make_async_copy(vbuf.at[slot], vbuf.at[slot], kvsem.at[1, si]).wait()

        wcopies = [
            pltpu.make_async_copy(x_hbm, x_v, wsem.at[0]),
            pltpu.make_async_copy(wq_hbm, wq_v, wsem.at[1]),
            pltpu.make_async_copy(wo_hbm, wo_v, wsem.at[2]),
            pltpu.make_async_copy(w1_hbm, w1_v, wsem.at[3]),
            pltpu.make_async_copy(w2_hbm, w2_v, wsem.at[4]),
            pltpu.make_async_copy(b1_hbm, b1_v, wsem.at[5]),
        ]
        wcopies[0].start()
        wcopies[1].start()
        start(0, 0, 0)
        start(1, 1, 1)
        wcopies[0].wait()
        wcopies[1].wait()

        rows = lax.broadcasted_iota(jnp.int32, (8, _DH), 0)

        def make_q(x):
            xn = jnp.broadcast_to(_layernorm(x), (8, _D)).astype(jnp.bfloat16)
            y = jnp.dot(xn, wq_v[...], preferred_element_type=jnp.float32)
            for g in range(_HKV):
                t = jnp.zeros((8, _DH), jnp.float32)
                for j in range(4):
                    h = 4 * g + j
                    t = jnp.where(rows == 4 * (g % 2) + j, y[:, h * _DH:(h + 1) * _DH], t)
                q_scr[g] = t.astype(jnp.bfloat16)

        def compute(slot, carry):
            m, l, acc = carry
            ss = [lax.dot_general(q_scr[h], kbuf[slot, h], nt, preferred_element_type=jnp.float32)
                  for h in range(_HKV)]
            s = jnp.concatenate([ss[2 * j] + ss[2 * j + 1] for j in range(_HKV // 2)], axis=0) * scale
            mn = jnp.maximum(m, jnp.max(s, axis=1, keepdims=True))
            al = jnp.exp(m - mn)
            p = jnp.exp(s - mn)
            nl = al * l + jnp.sum(p, axis=1, keepdims=True)
            pb = p.astype(jnp.bfloat16)
            pv = [jnp.dot(pb[8 * (h // 2):8 * (h // 2) + 8], vbuf[slot, h], preferred_element_type=jnp.float32)
                  for h in range(_HKV)]
            pvc = jnp.concatenate([jnp.where(rows < 4, pv[2 * j], pv[2 * j + 1]) for j in range(_HKV // 2)], axis=0)
            return mn, nl, acc * al + pvc

        def init():
            return (jnp.full((_HQ, 1), -1e30, jnp.float32), jnp.zeros((_HQ, 1), jnp.float32),
                    jnp.zeros((_HQ, _DH), jnp.float32))

        def finish(x, carry):
            m, l, acc = carry
            o = acc / l
            blocks = []
            for h in range(_HQ):
                j = h // 8
                blocks.append(jnp.where(rows == h % 8, o[8 * j:8 * j + 8], 0.0).astype(jnp.bfloat16))
            a = jnp.concatenate(blocks, axis=1)
            y = jnp.dot(a, wo_v[...], preferred_element_type=jnp.float32)
            x = x + jnp.sum(y, axis=0, keepdims=True)
            xn = jnp.broadcast_to(_layernorm(x), (8, _D)).astype(jnp.bfloat16)
            hh = jnp.dot(xn, w1_v[...], preferred_element_type=jnp.float32)
            hh = hh + b1_v[...].astype(jnp.float32)
            sp = jnp.log1p(jnp.exp(-jnp.abs(hh))) + jnp.maximum(hh, 0.0)
            act = hh * jnp.tanh(sp)
            y2 = jnp.dot(act.astype(jnp.bfloat16), w2_v[...], preferred_element_type=jnp.float32)
            return x + y2[0:1, :]

        x = x_v[0].astype(jnp.float32)
        make_q(x)
        for i in range(2, NS):
            start(i, i, i)
        for c in wcopies[2:]:
            c.start()

        def body1(s, carry):
            si = lax.rem(s, NS)
            slot = lax.rem(s, N)
            wait(slot, si)

            @pl.when(s + NS < T)
            def _():
                start(s + NS, lax.rem(s + NS, N), si)
            return compute(slot, carry)

        carry = lax.fori_loop(0, T, body1, init(), unroll=UNROLL)
        for c in wcopies[2:]:
            c.wait()
        x = finish(x, carry)
        make_q(x)

        def body2(c, carry):
            def w_of(c):
                pace = jnp.where(c >= NS + 1, lax.div(jnp.maximum(c - NS - 1, 0), RHO) + 1, 0)
                return jnp.minimum(jnp.maximum(pace, c - N + 1), ND)
            w1 = w_of(c)
            w0 = w_of(c - 1)

            @pl.when(w1 > w0)
            def _():
                n = w1 - 1
                si = lax.rem(n, NS)
                wait(lax.rem(T + n, N), si)

                @pl.when(n + NS < ND)
                def _():
                    start(n + NS, lax.rem(T + n + NS, N), si)
            slot = lax.rem(T + c, N)
            carry = compute(slot, carry)

            @pl.when(c < NS)
            def _():
                start(c, slot, c)
            return carry

        carry = lax.fori_loop(0, T, body2, init(), unroll=UNROLL)
        x = finish(x, carry)
        o_ref[0] = x.astype(o_ref.dtype)

    return kernel, N, NS, SB


def _build(**kw):
    kernel, N, NS, SB = make_kernel(**kw)

    def f(A_x, A_k_cache, A_v_cache, A_wq, A_wo, B_x, B_w1, B_b1, B_w2):
        k = A_k_cache.reshape(_HKV, _SK, _DH)
        v = A_v_cache.reshape(_HKV, _SK, _DH)
        b1 = B_b1.reshape(1, _F)
        hbm = pl.BlockSpec(memory_space=pltpu.HBM)
        return pl.pallas_call(
            kernel,
            out_shape=jax.ShapeDtypeStruct((1, 1, _D), A_x.dtype),
            in_specs=[hbm] * 8,
            out_specs=pl.BlockSpec(memory_space=pltpu.VMEM),
            scratch_shapes=[
                pltpu.VMEM((N, _HKV, SB, _DH), jnp.bfloat16),
                pltpu.VMEM((N, _HKV, SB, _DH), jnp.bfloat16),
                pltpu.VMEM((_D, _HQ * _DH), jnp.bfloat16),
                pltpu.VMEM((_HQ * _DH, _D), jnp.bfloat16),
                pltpu.VMEM((_D, _F), jnp.bfloat16),
                pltpu.VMEM((_F, _D), jnp.bfloat16),
                pltpu.VMEM((1, _F), jnp.bfloat16),
                pltpu.VMEM((1, 1, _D), jnp.bfloat16),
                pltpu.VMEM((_HKV, 8, _DH), jnp.bfloat16),
                pltpu.SemaphoreType.DMA((2, NS)),
                pltpu.SemaphoreType.DMA((6,)),
            ],
            compiler_params=pltpu.CompilerParams(vmem_limit_bytes=128 * 1024 * 1024),
        )(A_x, k, v, A_wq, A_wo, B_w1, b1, B_w2)
    return f


@jax.jit
def pallas_interleave_layers__gqa_block_cached__dense_activation_mish__decode_kernel(
    A_x, A_k_cache, A_v_cache, A_wq, A_wo, B_x, B_w1, B_b1, B_w2,
):
    return _build()(A_x, A_k_cache, A_v_cache, A_wq, A_wo, B_x, B_w1, B_b1, B_w2)
```

```python
import jax
import jax.numpy as jnp
from jax import lax
from jax.experimental import pallas as pl
from jax.experimental.pallas import tpu as pltpu

_D = 512
_HQ = 32
_HKV = 8
_DH = 128
_F = 1792
_SK = 65536
_NP = 4

_SB = 256
_T = _SK // _SB
_N = 116
_ND = _T - _N
_NS = 4
_DSB = 64
_I2 = _N - 6
_S0 = _T - _NP
_SCALE = float(_DH) ** -0.5
_NT = (((1,), (1,)), ((), ()))

assert _NS == _NP and 2 * _I2 + 6 - _N == _I2
assert 2 * _I2 + 6 <= _T - _NP and _I2 + _NS <= _ND - _NP


def _layernorm(x):
    m = jnp.mean(x, axis=-1, keepdims=True)
    xc = x - m
    v = jnp.mean(xc * xc, axis=-1, keepdims=True)
    return xc / jnp.sqrt(v + 1e-5)


def _kernel(x_hbm, k_hbm, v_hbm, wq_hbm, wo_hbm, w1_hbm, b1_hbm, w2_hbm,
            o_ref,
            kbuf, vbuf, wq_v, wo_v, w1_v, w2_v, b1_v, x_v, q_scr, m_s, l_s, acc_s,
            kvsem, wsem, bar_sem):
    f32, bf16 = jnp.float32, jnp.bfloat16

    def _start_piece(h0, s0, slot, a, b, si):
        pltpu.make_async_copy(
            k_hbm.at[pl.ds(h0, 2), pl.ds(s0, _DSB)],
            kbuf.at[slot, pl.ds(2 * a, 2), pl.ds(b * _DSB, _DSB)],
            kvsem.at[0, si]).start(priority=0)
        pltpu.make_async_copy(
            v_hbm.at[pl.ds(h0, 2), pl.ds(s0, _DSB)],
            vbuf.at[slot, pl.ds(2 * a, 2), pl.ds(b * _DSB, _DSB)],
            kvsem.at[1, si]).start(priority=1)

    def start_normal(blk, slot, si):
        s0 = blk * _SB
        for b in range(_SB // _DSB):
            for a in range(_NP):
                _start_piece(2 * a, s0 + b * _DSB, slot, a, b, si)

    def start_special(j, key0, slot, si):
        for a in range(_NP):
            for b in range(_SB // _DSB):
                _start_piece(2 * j, key0 + a * _SB + b * _DSB, slot, a, b, si)

    def start(n, nblk, slot, si):
        @pl.when(n < nblk - _NP)
        def _():
            start_normal(n, slot, si)

        @pl.when(n >= nblk - _NP)
        def _():
            start_special(n - (nblk - _NP), (nblk - _NP) * _SB, slot, si)

    def wait(slot, si):
        pltpu.make_async_copy(kbuf.at[slot], kbuf.at[slot], kvsem.at[0, si]).wait()
        pltpu.make_async_copy(vbuf.at[slot], vbuf.at[slot], kvsem.at[1, si]).wait()

    def start_weights(src, dst, sem, r, c):
        nr, nc = src.shape[0] // r, src.shape[1] // c
        half = nr * nc // 2

        def body(i, carry):
            for p in range(2):
                t = i + p * half
                r0 = pl.multiple_of(lax.div(t, nc) * r, r)
                c0 = pl.multiple_of(lax.rem(t, nc) * c, c)
                pltpu.make_async_copy(src.at[pl.ds(r0, r), pl.ds(c0, c)],
                                      dst.at[pl.ds(r0, r), pl.ds(c0, c)], sem).start(priority=p)
            return carry
        lax.fori_loop(0, half, body, 0)

    def wait_weights(dst, sem):
        pltpu.make_async_copy(dst, dst, sem).wait()

    rows = lax.broadcasted_iota(jnp.int32, (8, _DH), 0)

    def sel(a, b):
        return jnp.where(rows < 4, a, b)

    def rep(m):
        return jnp.concatenate([m] * (_SB // _DH), axis=1)

    def norm_bcast(x):
        return jnp.broadcast_to(_layernorm(x), (8, _D)).astype(bf16)

    def make_q_all(xn):
        y = jnp.dot(xn, wq_v[...], preferred_element_type=f32)
        for g in range(_HKV):
            t = jnp.zeros((8, _DH), f32)
            for i in range(4):
                h = 4 * g + i
                t = jnp.where(rows == 4 * (g % 2) + i, y[:, h * _DH:(h + 1) * _DH], t)
            q_scr[g] = t.astype(bf16)

    def make_q_pair(xn, j):
        c0 = pl.multiple_of(j * (8 * _DH), 8 * _DH)
        y = jnp.dot(xn, wq_v[:, pl.ds(c0, 8 * _DH)], preferred_element_type=f32)
        for g in range(2):
            t = jnp.zeros((8, _DH), f32)
            for i in range(4):
                h = 4 * g + i
                t = jnp.where(rows == h, y[:, h * _DH:(h + 1) * _DH], t)
            q_scr[2 * j + g] = t.astype(bf16)

    def reset_state():
        m_s[...] = jnp.full(m_s.shape, -jnp.inf, f32)
        l_s[...] = jnp.zeros(l_s.shape, f32)
        acc_s[...] = jnp.zeros(acc_s.shape, f32)

    def attend(slots):
        ss = [[lax.dot_general(q_scr[h], kbuf[sl, h], _NT, preferred_element_type=f32)
               for h in range(_HKV)] for sl in slots]
        ss = [[(s[2 * j] + s[2 * j + 1]) * _SCALE for j in range(_NP)] for s in ss]
        ms = [m_s[j] for j in range(_NP)]
        mn = []
        for j in range(_NP):
            mx = ss[0][j]
            for s in ss[1:]:
                mx = jnp.maximum(mx, s[j])
            mn.append(jnp.maximum(ms[j], jnp.max(mx, axis=1, keepdims=True)))
        al = [jnp.exp(ms[j] - mn[j]) for j in range(_NP)]
        mr = [rep(m) for m in mn]
        ps = [[jnp.exp(s[j] - mr[j]) for j in range(_NP)] for s in ss]
        pb = [[p.astype(bf16) for p in pp] for pp in ps]
        for j in range(_NP):
            psum = ps[0][j]
            for pp in ps[1:]:
                psum = psum + pp[j]
            m_s[j] = mn[j]
            l_s[j] = al[j] * l_s[j] + jnp.sum(psum, axis=1, keepdims=True)
        pv = [[jnp.dot(pb[i][h // 2], vbuf[sl, h], preferred_element_type=f32)
               for h in range(_HKV)] for i, sl in enumerate(slots)]
        for j in range(_NP):
            a, b = pv[0][2 * j], pv[0][2 * j + 1]
            for p in pv[1:]:
                a, b = a + p[2 * j], b + p[2 * j + 1]
            acc_s[j] = acc_s[j] * al[j] + sel(a, b)

    def attend_pair(j, slot):
        ss = [lax.dot_general(q_scr[2 * j + (h % 2)], kbuf[slot, h], _NT, preferred_element_type=f32)
              for h in range(_HKV)]
        ss = [(ss[2 * c] + ss[2 * c + 1]) * _SCALE for c in range(_NP)]
        mc = [jnp.max(ss[c], axis=1, keepdims=True) for c in range(_NP)]
        ps = [jnp.exp(ss[c] - rep(jnp.broadcast_to(mc[c], (8, _DH)))) for c in range(_NP)]
        pb = [p.astype(bf16) for p in ps]
        lc = [jnp.sum(ps[c], axis=1, keepdims=True) for c in range(_NP)]
        pv = [jnp.dot(pb[h // 2], vbuf[slot, h], preferred_element_type=f32) for h in range(_HKV)]
        m0 = m_s[j]
        mn = jnp.maximum(m0, jnp.maximum(jnp.maximum(mc[0], mc[1]), jnp.maximum(mc[2], mc[3])))
        al = jnp.exp(m0 - mn)
        bc = [jnp.exp(mc[c] - mn) for c in range(_NP)]
        m_s[j] = mn
        l_s[j] = al * l_s[j] + ((bc[0] * lc[0] + bc[1] * lc[1]) + (bc[2] * lc[2] + bc[3] * lc[3]))
        acc = acc_s[j] * al
        for c in range(_NP):
            acc = acc + bc[c] * sel(pv[2 * c], pv[2 * c + 1])
        acc_s[j] = acc

    def oproj(j):
        o = acc_s[j] / l_s[j]
        a = jnp.concatenate([jnp.where(rows == r, o, 0.0).astype(bf16) for r in range(8)], axis=1)
        r0 = pl.multiple_of(j * (8 * _DH), 8 * _DH)
        return jnp.dot(a, wo_v[pl.ds(r0, 8 * _DH), :], preferred_element_type=f32)

    def ffn(x):
        h = jnp.dot(norm_bcast(x), w1_v[...], preferred_element_type=f32)
        h = h + b1_v[...].reshape(1, _F).astype(f32)
        sp = jnp.log1p(jnp.exp(-jnp.abs(h))) + jnp.maximum(h, 0.0)
        act = h * jnp.tanh(sp)
        y = jnp.dot(act.astype(bf16), w2_v[...], preferred_element_type=f32)
        return x + y[0:1, :]

    def endgame(x, step0, n0):
        def body(j, y):
            slot = lax.rem(step0 + j, _N)
            wait(slot, lax.rem(n0 + j, _NS))
            attend_pair(j, slot)
            return y + oproj(j)
        y = lax.fori_loop(0, _NP, body, jnp.zeros((8, _D), f32))
        return ffn(x + jnp.sum(y, axis=0, keepdims=True))

    x_cp = pltpu.make_async_copy(x_hbm, x_v, wsem.at[0])
    b1_cp = pltpu.make_async_copy(b1_hbm, b1_v, wsem.at[5])
    x_cp.start()
    start_weights(wq_hbm, wq_v, wsem.at[1], 16, 512)
    start_normal(0, 0, 0)
    start_normal(1, 1, 1)
    x_cp.wait()
    wait_weights(wq_v, wsem.at[1])
    x = x_v[0].astype(f32)
    make_q_all(norm_bcast(x))
    for i in range(2, _NS):
        start_normal(i, i, i)
    b1_cp.start()
    start_weights(wo_hbm, wo_v, wsem.at[2], 16, 512)
    start_weights(w1_hbm, w1_v, wsem.at[3], 16, 896)
    start_weights(w2_hbm, w2_v, wsem.at[4], 16, 512)
    reset_state()

    def body1(s, carry):
        si = lax.rem(s, _NS)
        slot = lax.rem(s, _N)
        wait(slot, si)

        @pl.when(s + _NS < _T)
        def _():
            start(s + _NS, _T, lax.rem(s + _NS, _N), si)
        attend((slot,))
        return carry

    lax.fori_loop(0, _T - _NP, body1, 0)
    b1_cp.wait()
    wait_weights(wo_v, wsem.at[2])
    wait_weights(w1_v, wsem.at[3])
    wait_weights(w2_v, wsem.at[4])
    x = endgame(x, _T - _NP, _T - _NP)

    reset_state()
    xn = norm_bcast(x)

    def head2(c, carry):
        slot = lax.rem(_S0 + c, _N)
        make_q_pair(xn, c)
        pl.semaphore_signal(bar_sem, 1)
        pl.semaphore_wait(bar_sem, 1)
        attend_pair(c, slot)
        start_normal(c, slot, c)
        return carry

    lax.fori_loop(0, _NP, head2, 0)
    attend(((_S0 + 4) % _N, (_S0 + 5) % _N))

    def body2a(i, carry):
        si = lax.rem(i, _NS)
        wait(lax.rem(_S0 + i, _N), si)
        start_normal(i + _NS, lax.rem(_S0 + i + _NS, _N), si)
        c = 2 * i + 6
        attend((lax.rem(_S0 + c, _N), lax.rem(_S0 + c + 1, _N)))
        return carry

    lax.fori_loop(0, _I2, body2a, 0)

    def body2b(n, carry):
        si = lax.rem(n, _NS)
        slot = lax.rem(_S0 + n, _N)
        wait(slot, si)
        start(n + _NS, _ND, lax.rem(_S0 + n + _NS, _N), si)
        attend((slot,))
        return carry

    lax.fori_loop(_I2, _ND - _NP, body2b, 0)
    x = endgame(x, _S0 + _T - _NP, _ND - _NP)
    o_ref[0] = x.astype(o_ref.dtype)


@jax.jit
def pallas_interleave_layers__gqa_block_cached__dense_activation_mish__decode_kernel(
    A_x: jax.Array,
    A_k_cache: jax.Array,
    A_v_cache: jax.Array,
    A_wq: jax.Array,
    A_wo: jax.Array,
    B_x: jax.Array,
    B_w1: jax.Array,
    B_b1: jax.Array,
    B_w2: jax.Array,
):
    del B_x
    k = A_k_cache.reshape(_HKV, _SK, _DH)
    v = A_v_cache.reshape(_HKV, _SK, _DH)
    hbm = pl.BlockSpec(memory_space=pltpu.HBM)
    bf16, f32 = jnp.bfloat16, jnp.float32
    return pl.pallas_call(
        _kernel,
        out_shape=jax.ShapeDtypeStruct((1, 1, _D), A_x.dtype),
        in_specs=[hbm] * 8,
        out_specs=pl.BlockSpec(memory_space=pltpu.VMEM),
        scratch_shapes=[
            pltpu.VMEM((_N, _HKV, _SB, _DH), bf16),
            pltpu.VMEM((_N, _HKV, _SB, _DH), bf16),
            pltpu.VMEM((_D, _HQ * _DH), bf16),
            pltpu.VMEM((_HQ * _DH, _D), bf16),
            pltpu.VMEM((_D, _F), bf16),
            pltpu.VMEM((_F, _D), bf16),
            pltpu.VMEM((_F,), bf16),
            pltpu.VMEM((1, 1, _D), bf16),
            pltpu.VMEM((_HKV, 8, _DH), bf16),
            pltpu.VMEM((_NP, 8, _DH), f32),
            pltpu.VMEM((_NP, 8, _DH), f32),
            pltpu.VMEM((_NP, 8, _DH), f32),
            pltpu.SemaphoreType.DMA((2, _NS)),
            pltpu.SemaphoreType.DMA((6,)),
            pltpu.SemaphoreType.REGULAR,
        ],
        compiler_params=pltpu.CompilerParams(vmem_limit_bytes=128 * 1024 * 1024),
    )(A_x, k, v, A_wq, A_wo, B_w1, B_b1, B_w2)
```

```python
import jax
import jax.numpy as jnp
from jax import lax
from jax.experimental import pallas as pl
from jax.experimental.pallas import tpu as pltpu

_D = 512
_HQ = 32
_HKV = 8
_DH = 128
_F = 1792
_SK = 65536
_NP = 4

_SB = 256
_T = _SK // _SB
_N = 116
_X = _T - _N - 1
_ND = _T - _N - 1
_PV = 6
_NS = 4
_DSB = 64
_I2 = _N - 5
_S0 = _T - _NP
_SCALE = float(_DH) ** -0.5
_NT = (((1,), (1,)), ((), ()))

assert _NS == _NP and 2 * _I2 + 6 - _N - 1 == _I2
assert 2 * _I2 + 6 <= _T - _NP and _I2 + _NS <= _ND - _NP


def _layernorm(x):
    m = jnp.mean(x, axis=-1, keepdims=True)
    xc = x - m
    v = jnp.mean(xc * xc, axis=-1, keepdims=True)
    return xc / jnp.sqrt(v + 1e-5)


def _kernel(x_hbm, k_hbm, v_hbm, wq_hbm, wo_hbm, w1_hbm, b1_hbm, w2_hbm,
            o_ref,
            kbuf, vbuf, wq_v, wo_v, w1_v, w2_v, b1_v, x_v, q_scr, m_s, l_s, acc_s,
            kvsem, wsem, bar_sem, k_park, v_park, psem):
    f32, bf16 = jnp.float32, jnp.bfloat16

    def _start_piece(h0, s0, slot, a, b, si):
        pltpu.make_async_copy(
            k_hbm.at[pl.ds(h0, 2), pl.ds(s0, _DSB)],
            kbuf.at[slot, pl.ds(2 * a, 2), pl.ds(b * _DSB, _DSB)],
            kvsem.at[0, si]).start(priority=0)
        pltpu.make_async_copy(
            v_hbm.at[pl.ds(h0, 2), pl.ds(s0, _DSB)],
            vbuf.at[slot, pl.ds(2 * a, 2), pl.ds(b * _DSB, _DSB)],
            kvsem.at[1, si]).start(priority=1)

    def start_normal(blk, slot, si):
        s0 = blk * _SB
        for b in range(_SB // _DSB):
            for a in range(_NP):
                _start_piece(2 * a, s0 + b * _DSB, slot, a, b, si)

    def start_special(j, key0, slot, si):
        for a in range(_NP):
            for b in range(_SB // _DSB):
                _start_piece(2 * j, key0 + a * _SB + b * _DSB, slot, a, b, si)

    def start(n, nblk, slot, si):
        @pl.when(n < nblk - _NP)
        def _():
            start_normal(n, slot, si)

        @pl.when(n >= nblk - _NP)
        def _():
            start_special(n - (nblk - _NP), (nblk - _NP) * _SB, slot, si)

    def wait(slot, si):
        pltpu.make_async_copy(kbuf.at[slot], kbuf.at[slot], kvsem.at[0, si]).wait()
        pltpu.make_async_copy(vbuf.at[slot], vbuf.at[slot], kvsem.at[1, si]).wait()

    def park_copies(slot, restore):
        pairs = [(kbuf.at[slot], k_park), (vbuf.at[slot, pl.ds(0, _PV)], v_park)]
        if restore:
            pairs = [(b, a) for a, b in pairs]
            pairs.append((v_hbm.at[pl.ds(_PV, _HKV - _PV), pl.ds(_X * _SB, _SB)],
                          vbuf.at[slot, pl.ds(_PV, _HKV - _PV)]))
        return [pltpu.make_async_copy(a, b, psem.at[i]) for i, (a, b) in enumerate(pairs)]

    def start_weights(src, dst, sem, r, c):
        nr, nc = src.shape[0] // r, src.shape[1] // c
        half = nr * nc // 2

        def body(i, carry):
            for p in range(2):
                t = i + p * half
                r0 = pl.multiple_of(lax.div(t, nc) * r, r)
                c0 = pl.multiple_of(lax.rem(t, nc) * c, c)
                pltpu.make_async_copy(src.at[pl.ds(r0, r), pl.ds(c0, c)],
                                      dst.at[pl.ds(r0, r), pl.ds(c0, c)], sem).start(priority=p)
            return carry
        lax.fori_loop(0, half, body, 0)

    def wait_weights(dst, sem):
        pltpu.make_async_copy(dst, dst, sem).wait()

    rows = lax.broadcasted_iota(jnp.int32, (8, _DH), 0)

    def sel(a, b):
        return jnp.where(rows < 4, a, b)

    def rep(m):
        return jnp.concatenate([m] * (_SB // _DH), axis=1)

    def norm_bcast(x):
        return jnp.broadcast_to(_layernorm(x), (8, _D)).astype(bf16)

    def make_q_all(xn):
        y = jnp.dot(xn, wq_v[...], preferred_element_type=f32)
        for g in range(_HKV):
            t = jnp.zeros((8, _DH), f32)
            for i in range(4):
                h = 4 * g + i
                t = jnp.where(rows == 4 * (g % 2) + i, y[:, h * _DH:(h + 1) * _DH], t)
            q_scr[g] = t.astype(bf16)

    def make_q_pair(xn, j):
        c0 = pl.multiple_of(j * (8 * _DH), 8 * _DH)
        y = jnp.dot(xn, wq_v[:, pl.ds(c0, 8 * _DH)], preferred_element_type=f32)
        for g in range(2):
            t = jnp.zeros((8, _DH), f32)
            for i in range(4):
                h = 4 * g + i
                t = jnp.where(rows == h, y[:, h * _DH:(h + 1) * _DH], t)
            q_scr[2 * j + g] = t.astype(bf16)

    def reset_state():
        m_s[...] = jnp.full(m_s.shape, -jnp.inf, f32)
        l_s[...] = jnp.zeros(l_s.shape, f32)
        acc_s[...] = jnp.zeros(acc_s.shape, f32)

    def attend(slots):
        ss = [[lax.dot_general(q_scr[h], kbuf[sl, h], _NT, preferred_element_type=f32)
               for h in range(_HKV)] for sl in slots]
        ss = [[(s[2 * j] + s[2 * j + 1]) * _SCALE for j in range(_NP)] for s in ss]
        ms = [m_s[j] for j in range(_NP)]
        mn = []
        for j in range(_NP):
            mx = ss[0][j]
            for s in ss[1:]:
                mx = jnp.maximum(mx, s[j])
            mn.append(jnp.maximum(ms[j], jnp.max(mx, axis=1, keepdims=True)))
        al = [jnp.exp(ms[j] - mn[j]) for j in range(_NP)]
        mr = [rep(m) for m in mn]
        ps = [[jnp.exp(s[j] - mr[j]) for j in range(_NP)] for s in ss]
        pb = [[p.astype(bf16) for p in pp] for pp in ps]
        for j in range(_NP):
            psum = ps[0][j]
            for pp in ps[1:]:
                psum = psum + pp[j]
            m_s[j] = mn[j]
            l_s[j] = al[j] * l_s[j] + jnp.sum(psum, axis=1, keepdims=True)
        pv = [[jnp.dot(pb[i][h // 2], vbuf[sl, h], preferred_element_type=f32)
               for h in range(_HKV)] for i, sl in enumerate(slots)]
        for j in range(_NP):
            a, b = pv[0][2 * j], pv[0][2 * j + 1]
            for p in pv[1:]:
                a, b = a + p[2 * j], b + p[2 * j + 1]
            acc_s[j] = acc_s[j] * al[j] + sel(a, b)

    def attend_pair(j, slot):
        ss = [lax.dot_general(q_scr[2 * j + (h % 2)], kbuf[slot, h], _NT, preferred_element_type=f32)
              for h in range(_HKV)]
        ss = [(ss[2 * c] + ss[2 * c + 1]) * _SCALE for c in range(_NP)]
        mc = [jnp.max(ss[c], axis=1, keepdims=True) for c in range(_NP)]
        ps = [jnp.exp(ss[c] - rep(jnp.broadcast_to(mc[c], (8, _DH)))) for c in range(_NP)]
        pb = [p.astype(bf16) for p in ps]
        lc = [jnp.sum(ps[c], axis=1, keepdims=True) for c in range(_NP)]
        pv = [jnp.dot(pb[h // 2], vbuf[slot, h], preferred_element_type=f32) for h in range(_HKV)]
        m0 = m_s[j]
        mn = jnp.maximum(m0, jnp.maximum(jnp.maximum(mc[0], mc[1]), jnp.maximum(mc[2], mc[3])))
        al = jnp.exp(m0 - mn)
        bc = [jnp.exp(mc[c] - mn) for c in range(_NP)]
        m_s[j] = mn
        l_s[j] = al * l_s[j] + ((bc[0] * lc[0] + bc[1] * lc[1]) + (bc[2] * lc[2] + bc[3] * lc[3]))
        acc = acc_s[j] * al
        for c in range(_NP):
            acc = acc + bc[c] * sel(pv[2 * c], pv[2 * c + 1])
        acc_s[j] = acc

    def oproj(j):
        o = acc_s[j] / l_s[j]
        a = jnp.concatenate([jnp.where(rows == r, o, 0.0).astype(bf16) for r in range(8)], axis=1)
        r0 = pl.multiple_of(j * (8 * _DH), 8 * _DH)
        return jnp.dot(a, wo_v[pl.ds(r0, 8 * _DH), :], preferred_element_type=f32)

    def ffn(x):
        h = jnp.dot(norm_bcast(x), w1_v[...], preferred_element_type=f32)
        h = h + b1_v[...].reshape(1, _F).astype(f32)
        sp = jnp.log1p(jnp.exp(-jnp.abs(h))) + jnp.maximum(h, 0.0)
        act = h * jnp.tanh(sp)
        y = jnp.dot(act.astype(bf16), w2_v[...], preferred_element_type=f32)
        return x + y[0:1, :]

    def endgame(x, step0, n0):
        def body(j, y):
            slot = lax.rem(step0 + j, _N)
            wait(slot, lax.rem(n0 + j, _NS))
            attend_pair(j, slot)
            return y + oproj(j)
        y = lax.fori_loop(0, _NP, body, jnp.zeros((8, _D), f32))
        return ffn(x + jnp.sum(y, axis=0, keepdims=True))

    x_cp = pltpu.make_async_copy(x_hbm, x_v, wsem.at[0])
    b1_cp = pltpu.make_async_copy(b1_hbm, b1_v, wsem.at[5])
    x_cp.start()
    start_weights(wq_hbm, wq_v, wsem.at[1], 16, 512)
    start_normal(0, 0, 0)
    start_normal(1, 1, 1)
    x_cp.wait()
    wait_weights(wq_v, wsem.at[1])
    x = x_v[0].astype(f32)
    make_q_all(norm_bcast(x))
    for i in range(2, _NS):
        start_normal(i, i, i)
    b1_cp.start()
    start_weights(wo_hbm, wo_v, wsem.at[2], 16, 512)
    start_weights(w1_hbm, w1_v, wsem.at[3], 16, 896)
    start_weights(w2_hbm, w2_v, wsem.at[4], 16, 512)
    reset_state()

    def body1(s, carry):
        si = lax.rem(s, _NS)
        slot = lax.rem(s, _N)
        wait(slot, si)

        @pl.when(s + _NS < _T)
        def _():
            start(s + _NS, _T, lax.rem(s + _NS, _N), si)
        attend((slot,))

        @pl.when(s == _X)
        def _():
            for c in park_copies(slot, False):
                c.start()

        @pl.when(s == _X + _N - 2 * _NS)
        def _():
            for c in park_copies(_X % _N, False):
                c.wait()
        return carry

    lax.fori_loop(0, _T - _NP, body1, 0)
    b1_cp.wait()
    wait_weights(wo_v, wsem.at[2])
    wait_weights(w1_v, wsem.at[3])
    wait_weights(w2_v, wsem.at[4])
    x = endgame(x, _T - _NP, _T - _NP)

    reset_state()
    xn = norm_bcast(x)

    def head2(c, carry):
        slot = lax.rem(_S0 + c, _N)
        make_q_pair(xn, c)
        pl.semaphore_signal(bar_sem, 1)
        pl.semaphore_wait(bar_sem, 1)
        attend_pair(c, slot)
        start_normal(c, slot, c)
        return carry

    lax.fori_loop(0, _NP, head2, 0)
    attend(((_S0 + 4) % _N, (_S0 + 5) % _N))
    for c in park_copies((_S0 + 4) % _N, True):
        c.start()

    def dslot(n):
        return lax.rem(_S0 + n + jnp.where(n >= _NP, 1, 0), _N)

    def body2a(i, carry):
        si = lax.rem(i, _NS)
        wait(dslot(i), si)
        start_normal(i + _NS, dslot(i + _NS), si)
        c = 2 * i + 6
        attend((lax.rem(_S0 + c, _N), lax.rem(_S0 + c + 1, _N)))
        return carry

    ip = (_N - 2) // 2
    lax.fori_loop(0, ip, body2a, 0)
    for c in park_copies((_S0 + 4) % _N, True):
        c.wait()
    lax.fori_loop(ip, _I2, body2a, 0)

    def body2b(n, carry):
        si = lax.rem(n, _NS)
        slot = dslot(n)
        wait(slot, si)
        start(n + _NS, _ND, dslot(n + _NS), si)
        attend((slot,))
        return carry

    lax.fori_loop(_I2, _ND - _NP, body2b, 0)
    x = endgame(x, _S0 + _T - _NP, _ND - _NP)
    o_ref[0] = x.astype(o_ref.dtype)


@jax.jit
def pallas_interleave_layers__gqa_block_cached__dense_activation_mish__decode_kernel(
    A_x: jax.Array,
    A_k_cache: jax.Array,
    A_v_cache: jax.Array,
    A_wq: jax.Array,
    A_wo: jax.Array,
    B_x: jax.Array,
    B_w1: jax.Array,
    B_b1: jax.Array,
    B_w2: jax.Array,
):
    del B_x
    k = A_k_cache.reshape(_HKV, _SK, _DH)
    v = A_v_cache.reshape(_HKV, _SK, _DH)
    hbm = pl.BlockSpec(memory_space=pltpu.HBM)
    bf16, f32 = jnp.bfloat16, jnp.float32
    return pl.pallas_call(
        _kernel,
        out_shape=jax.ShapeDtypeStruct((1, 1, _D), A_x.dtype),
        in_specs=[hbm] * 8,
        out_specs=pl.BlockSpec(memory_space=pltpu.VMEM),
        scratch_shapes=[
            pltpu.VMEM((_N, _HKV, _SB, _DH), bf16),
            pltpu.VMEM((_N, _HKV, _SB, _DH), bf16),
            pltpu.VMEM((_D, _HQ * _DH), bf16),
            pltpu.VMEM((_HQ * _DH, _D), bf16),
            pltpu.VMEM((_D, _F), bf16),
            pltpu.VMEM((_F, _D), bf16),
            pltpu.VMEM((_F,), bf16),
            pltpu.VMEM((1, 1, _D), bf16),
            pltpu.VMEM((_HKV, 8, _DH), bf16),
            pltpu.VMEM((_NP, 8, _DH), f32),
            pltpu.VMEM((_NP, 8, _DH), f32),
            pltpu.VMEM((_NP, 8, _DH), f32),
            pltpu.SemaphoreType.DMA((2, _NS)),
            pltpu.SemaphoreType.DMA((6,)),
            pltpu.SemaphoreType.REGULAR,
            pltpu.SMEM((_HKV, _SB, _DH), bf16),
            pltpu.VMEM((_PV, _SB, _DH), bf16),
            pltpu.SemaphoreType.DMA((3,)),
        ],
        compiler_params=pltpu.CompilerParams(vmem_limit_bytes=128 * 1024 * 1024),
    )(A_x, k, v, A_wq, A_wo, B_w1, B_b1, B_w2)
```
